```python
import jax
import jax.numpy as jnp

def _softmax(x, axis=-1):
    return jax.nn.softmax(x, axis=axis)
def _gelu(x):
    return jax.nn.gelu(x, approximate=True)
def _silu(x):
    return jax.nn.silu(x)
def _sigmoid(x):
    return jax.nn.sigmoid(x)
def _layernorm(x, axis=-1, eps=1e-5):
    m = jnp.mean(x, axis=axis, keepdims=True)
    v = jnp.var(x, axis=axis, keepdims=True)
    return (x - m) / jnp.sqrt(v + eps)
def _scatter_add(tgt, idx, src, axis=0):
    return tgt.at[idx].add(src)
def _segment_sum(src, seg, n):
    return jax.ops.segment_sum(src, seg, n)
class _Rng:
    def __init__(self, key):
        self._k = key
    def _next(self):
        self._k, sub = jax.random.split(self._k)
        return sub
    def normal(self, shape):
        return jax.random.normal(self._next(), shape, dtype=jnp.bfloat16)
    def randint(self, lo, hi, shape):
        return jax.random.randint(self._next(), shape, lo, hi, dtype=jnp.int32)
    def uniform(self, shape, lo=0.0, hi=1.0):
        return jax.random.uniform(self._next(), shape, jnp.bfloat16, lo, hi)
    def permutation(self, n):
        return jax.random.permutation(self._next(), n)


kernel_name = 'parallel_sum__compressed_kv_cla__moe_arch_mod__prompt'

def setup_inputs():
    _rng = _Rng(jax.random.key(int.from_bytes(__import__("os").urandom(4), "little")))
    _w = (lambda a: (lambda t: t.astype(jnp.bfloat16) if jnp.issubdtype(t.dtype, jnp.floating) else t)(jnp.asarray(a)))
    def _A_setup():
        B, H, Sq, Sk, D, M = 1, 32, 2048, 2048, 128, 640
        Dc = 4 * D
        return {
            "x": _w((lambda *s: _rng.normal(s) * 0.05)(B, Sq, M)),
            "c_kv": _w((lambda *s: _rng.normal(s) * 0.05)(B, Sk, Dc)),
            "w_q": _w((lambda *s: _rng.normal(s) * 0.05)(M, H, D) * (M ** -0.5)),
            "w_uk": _w((lambda *s: _rng.normal(s) * 0.05)(Dc, H, D) * (Dc ** -0.5)),
            "w_uv": _w((lambda *s: _rng.normal(s) * 0.05)(Dc, H, D) * (Dc ** -0.5)),
            "w_o": _w((lambda *s: _rng.normal(s) * 0.05)(H, D, M) * ((H * D) ** -0.5)),
        }
    _A_in = _A_setup()

    def _B_setup():
        B, S, D, F, C = 1, 2048, 640, 1728, 8
        return {
            "x": _w((lambda *s: _rng.normal(s) * 0.05)(B, S, D)),
            "w_r": _w((lambda *s: _rng.normal(s) * 0.05)(D)),
            "w_gate": _w((lambda *s: _rng.normal(s) * 0.05)(D, F)),
            "w_up": _w((lambda *s: _rng.normal(s) * 0.05)(D, F)),
            "w_down": _w((lambda *s: _rng.normal(s) * 0.05)(F, D)),
        }
    _B_in = _B_setup()

    return {
        "A_x": _A_in["x"],
        "A_c_kv": _A_in["c_kv"],
        "A_w_q": _A_in["w_q"],
        "A_w_uk": _A_in["w_uk"],
        "A_w_uv": _A_in["w_uv"],
        "A_w_o": _A_in["w_o"],
        "B_x": _B_in["x"],
        "B_w_r": _B_in["w_r"],
        "B_w_gate": _B_in["w_gate"],
        "B_w_up": _B_in["w_up"],
        "B_w_down": _B_in["w_down"],
    }

def reference(A_x, A_c_kv, A_w_q, A_w_uk, A_w_uv, A_w_o, B_x, B_w_r, B_w_gate, B_w_up, B_w_down):
    def _A_ref(x, c_kv, w_q, w_uk, w_uv, w_o):
        B, Sq, M = x.shape[0], x.shape[1], x.shape[2]
        Sk = c_kv.shape[1]
        H, D = w_q.shape[1], w_q.shape[2]
        q = jnp.einsum("bqm,mhd->bhqd", x, w_q)
        k = jnp.einsum("bkc,chd->bhkd", c_kv, w_uk)
        v = jnp.einsum("bkc,chd->bhkd", c_kv, w_uv)
        scores = jnp.einsum("bhqd,bhkd->bhqk", q, k) * (D ** -0.5)
        off = Sk - Sq
        qi = jnp.arange(Sq)[:, None]
        kj = jnp.arange(Sk)[None, :]
        cmask = kj <= (qi + off)
        scores = jnp.where(cmask[None, None], scores, -1e9)
        p = _softmax(scores, axis=-1)
        ctx = jnp.einsum("bhqk,bhkd->bhqd", p, v)
        return jnp.einsum("bhqd,hdm->bqm", ctx, w_o)

    def _B_ref(x, w_r, w_gate, w_up, w_down):
        B, S, D = x.shape
        C = 8
        r = x @ w_r
        idx = jnp.argsort(-r, axis=-1)[:, :C]
        idx_e = jnp.repeat(idx.reshape(B, C, 1), D, axis=2)
        x_sel = jnp.take_along_axis(x, idx_e, axis=1)
        g = _silu(x_sel @ w_gate)
        u = x_sel @ w_up
        y = (g * u) @ w_down
        r_sel = _sigmoid(jnp.take_along_axis(r, idx, axis=1))
        y = y * r_sel.reshape(B, C, 1)
        b_off = (jnp.arange(B) * S).reshape(B, 1)
        flat_idx = (idx + b_off).reshape(B * C)
        zero = (x * 0.0).reshape(B * S, D)
        upd = _scatter_add(zero, flat_idx, y.reshape(B * C, D), axis=0)
        return x + upd.reshape(B, S, D)

    x = A_x
    xn = _layernorm(x, axis=-1)
    return x + _A_ref(xn, A_c_kv, A_w_q, A_w_uk, A_w_uv, A_w_o) + _B_ref(xn, B_w_r, B_w_gate, B_w_up, B_w_down)
```

```python
import functools
import math
import os
import jax
import jax.numpy as jnp
import numpy as np
from jax import lax
import jax.experimental.pallas as pl
import jax.experimental.pallas.tpu as pltpu

S, M, DC, H, D, F, C = 2048, 640, 512, 32, 128, 1728, 8
LOG2E = math.log2(math.e)
QSCALE = (D ** -0.5) * LOG2E
MASKV = -998244352.0 * LOG2E
EPS = 1.0013580322265625e-05
BQ = int(os.environ.get("BQ", "256"))
ORDER = os.environ.get("ORDER", "a")
NB = S // BQ
f32, bf16, u32 = jnp.float32, jnp.bfloat16, jnp.uint32
NT = (((1,), (1,)), ((), ()))


def _rb(x):
    return x.astype(bf16).astype(f32)


def _pk(x):
    return pltpu.bitcast(x.astype(bf16), u32)


def _ld(ref, r0, r1, cs=slice(None)):
    return pltpu.bitcast(ref[r0 // 2:r1 // 2, cs], bf16)


def _dot(a, b):
    return jnp.dot(a, b, preferred_element_type=f32)


def body(x_hbm, c_hbm, wq_hbm, wk_hbm, wv_hbm, wo_hbm, wr_hbm, wg_hbm, wu_hbm, wd_hbm, o_hbm,
         x_v, c_v, wq_v, wk_v, wv_v, wo_v, wr_v, wg_v, wu_v, wd_v, acc_v,
         xn_p, c_p, wq_p, wk_p, wv_p, wo_p, q_p, k_p, v_p, ctx_p, o_v, sem):
    cps = [pltpu.make_async_copy(s, d, sem.at[i]) for i, (s, d) in enumerate([
        (x_hbm, x_v), (c_hbm, c_v), (wk_hbm.bitcast(u32), wk_v), (wv_hbm.bitcast(u32), wv_v), (wq_hbm.bitcast(u32), wq_v), (wo_hbm, wo_v),
        (wr_hbm, wr_v), (wg_hbm, wg_v), (wu_hbm, wu_v), (wd_hbm, wd_v)])]
    for cp in cps[:6]:
        cp.start()
    cps[0].wait()
    cps[1].wait()

    def ln_body(i, _):
        r = pl.ds(pl.multiple_of(i * 256, 256), 256)
        rp = pl.ds(pl.multiple_of(i * 128, 128), 128)
        x = x_v[r, :].astype(f32)
        m = jnp.mean(x, axis=-1, keepdims=True)
        xc = x - m
        v = jnp.mean(xc * xc, axis=-1, keepdims=True)
        den = _rb(jnp.sqrt(_rb(_rb(v) + EPS)))
        xn_p[rp, :] = _pk(_rb(x - _rb(m)) / den)
        c_p[rp, :] = pltpu.bitcast(c_v[r, :], u32)
        acc_v[r, :] = jnp.zeros((256, M), f32)
        return _
    lax.fori_loop(0, S // 256, ln_body, None)
    for cp in cps[2:6]:
        cp.wait()
    for cp in cps[6:]:
        cp.start()

    def unpack_w(j, slot):
        for src, dst, n in ((wq_v, wq_p, M), (wk_v, wk_p, DC), (wv_v, wv_p, DC)):
            w = src[pl.ds(j, n, stride=H // 2), :]
            dst[slot, :, 0:D] = _pk(pltpu.bitcast(w << 16, f32))
            dst[slot, :, D:2 * D] = _pk(pltpu.bitcast(w & jnp.uint32(0xFFFF0000), f32))

    unpack_w(0, 0)
    tri = (lax.broadcasted_iota(jnp.int32, (D, D), 1) <= lax.broadcasted_iota(jnp.int32, (D, D), 0))

    def pair_body(j, _):
        slot = j % 2

        def proj(i):
            r0, r1 = i * BQ, (i + 1) * BQ
            wq = pltpu.bitcast(wq_p[slot], bf16)
            wk = pltpu.bitcast(wk_p[slot], bf16)
            wv = pltpu.bitcast(wv_p[slot], bf16)
            c = _ld(c_p, r0, r1)
            k_p[r0 // 2:r1 // 2, :] = _pk(_dot(c, wk))
            q_p[r0 // 2:r1 // 2, :] = _pk(_dot(_ld(xn_p, r0, r1), wq) * QSCALE)
            v_p[r0 // 2:r1 // 2, :] = _pk(_dot(c, wv))

        def qk(i, hh):
            r0, r1 = i * BQ, (i + 1) * BQ
            cs = slice(hh * D, (hh + 1) * D)
            nsub = BQ // D
            s0 = lax.dot_general(_ld(q_p, r0, r1, cs), _ld(k_p, 0, r0 + D, cs), NT, preferred_element_type=f32)
            sx = [lax.dot_general(_ld(q_p, r0 + t * D, r1, cs), _ld(k_p, r0 + t * D, r0 + (t + 1) * D, cs), NT,
                                  preferred_element_type=f32) for t in range(1, nsub)]
            return s0, sx

        def pv(i, hh, s):
            s0, sx = s
            r0, r1 = i * BQ, (i + 1) * BQ
            cs = slice(hh * D, (hh + 1) * D)
            nsub = BQ // D
            p0, px, ls = [], [[] for _ in range(1, nsub)], []
            for a in range(nsub):
                rs = slice(a * D, (a + 1) * D)
                if a == 0:
                    tiles = ([s0[rs, :r0]] if r0 else []) + [jnp.where(tri, s0[rs, r0:], MASKV)]
                else:
                    tiles = [s0[rs, :]] + [sx[t - 1][(a - t) * D:(a - t + 1) * D, :] for t in range(1, a)]
                    tiles.append(jnp.where(tri, sx[a - 1][0:D, :], MASKV))
                srow = jnp.concatenate(tiles, axis=1) if len(tiles) > 1 else tiles[0]
                m = jnp.max(srow, axis=-1, keepdims=True)
                p = jnp.exp2(srow - m)
                ls.append(jnp.sum(p, axis=-1, keepdims=True))
                p = p.astype(bf16)
                p0.append(p[:, :r0 + D])
                for t in range(1, a + 1):
                    px[t - 1].append(p[:, r0 + t * D:r0 + (t + 1) * D])
            o = _dot(jnp.concatenate(p0, axis=0), _ld(v_p, 0, r0 + D, cs))
            os_ = [o[a * D:(a + 1) * D] for a in range(nsub)]
            for t in range(1, nsub):
                pt = jnp.concatenate(px[t - 1], axis=0) if len(px[t - 1]) > 1 else px[t - 1][0]
                ot = _dot(pt, _ld(v_p, r0 + t * D, r0 + (t + 1) * D, cs))
                for a in range(t, nsub):
                    os_[a] = os_[a] + ot[(a - t) * D:(a - t + 1) * D]
            for a in range(nsub):
                ctx_p[(r0 + a * D) // 2:(r0 + (a + 1) * D) // 2, cs] = _pk(os_[a] * (1.0 / ls[a]))

        def oproj(i):
            r0, r1 = i * BQ, (i + 1) * BQ
            acc_v[r0:r1, :] += _dot(_ld(ctx_p, r0, r1), pltpu.bitcast(wo_p[...], bf16))

        proj(0)
        wo_p[...] = pltpu.bitcast(wo_v[pl.ds(pl.multiple_of(j * 2 * D, 2 * D), 2 * D), :], u32)
        for i in range(NB):
            if ORDER == "a":
                sa = qk(i, 0)
                sb = qk(i, 1)
                if i + 1 < NB:
                    proj(i + 1)
                pv(i, 0, sa)
                pv(i, 1, sb)
                if i > 0:
                    oproj(i - 1)
            elif ORDER == "b":
                if i + 1 < NB:
                    proj(i + 1)
                sa = qk(i, 0)
                sb = qk(i, 1)
                if i > 0:
                    oproj(i - 1)
                pv(i, 0, sa)
                pv(i, 1, sb)
            if i == 1:
                unpack_w(jnp.minimum(j + 1, H // 2 - 1), 1 - slot)
        oproj(NB - 1)
        return _
    lax.fori_loop(0, H // 2, pair_body, None)

    for cp in cps[6:]:
        cp.wait()
    xn = pltpu.bitcast(xn_p[...], bf16)
    wr = jnp.broadcast_to(wr_v[...], (8, M))
    r = lax.dot_general(wr, xn, NT, preferred_element_type=f32)
    r = _rb(r)
    lane = lax.broadcasted_iota(jnp.int32, (8, S), 1)
    sub = lax.broadcasted_iota(jnp.int32, (8, S), 0)
    cand = jnp.ones((8, S), jnp.int32)
    sel = jnp.zeros((8, S), f32)
    for i in range(C):
        rm = jnp.where(cand > 0, r, -jnp.inf)
        mx = jnp.max(rm, axis=-1, keepdims=True)
        idx = jnp.min(jnp.where((cand > 0) & (rm == mx), lane, S), axis=-1, keepdims=True)
        hit = lane == idx
        sel = jnp.where(hit & (sub == i), 1.0, sel)
        cand = jnp.where(hit, 0, cand)
    r_sel = jnp.sum(jnp.where(sel > 0, r, 0.0), axis=-1, keepdims=True)
    selb = sel.astype(bf16)
    xs = jnp.dot(selb, xn, preferred_element_type=f32).astype(bf16)
    g = _rb(lax.dot_general(xs, wg_v[...], NT, preferred_element_type=f32))
    u = _rb(lax.dot_general(xs, wu_v[...], NT, preferred_element_type=f32))
    g = _rb(g * _rb(jax.nn.sigmoid(g)))
    y = _rb(jnp.dot((g * u).astype(bf16), wd_v[...], preferred_element_type=f32))
    y = (y * _rb(jax.nn.sigmoid(r_sel))).astype(bf16)
    upd = lax.dot_general(selb, y, (((0,), (0,)), ((), ())), preferred_element_type=f32)
    a = _rb(x_v[...].astype(f32) + _rb(acc_v[...]))
    b = _rb(xn.astype(f32) + upd)
    o_v[...] = (a + b).astype(bf16)
    ocp = pltpu.make_async_copy(o_v, o_hbm, sem.at[0])
    ocp.start()
    ocp.wait()


@jax.jit
def pallas_parallel_sum__compressed_kv_cla__moe_arch_mod__prompt_kernel(
        A_x, A_c_kv, A_w_q, A_w_uk, A_w_uv, A_w_o, B_x, B_w_r, B_w_gate, B_w_up, B_w_down):
    del B_x
    V = pltpu.VMEM
    out = pl.pallas_call(
        body,
        in_specs=[pl.BlockSpec(memory_space=pltpu.HBM)] * 10,
        out_specs=pl.BlockSpec(memory_space=pltpu.HBM),
        out_shape=jax.ShapeDtypeStruct((S, M), bf16),
        scratch_shapes=[
            V((S, M), bf16), V((S, DC), bf16),
            V((M * H // 2, D), u32), V((DC * H // 2, D), u32), V((DC * H // 2, D), u32), V((H * D, M), bf16),
            V((1, M), bf16), V((F, M), bf16), V((F, M), bf16), V((F, M), bf16), V((S, M), f32),
            V((S // 2, M), u32), V((S // 2, DC), u32),
            V((2, M // 2, 2 * D), u32), V((2, DC // 2, 2 * D), u32), V((2, DC // 2, 2 * D), u32), V((D, M), u32),
            V((S // 2, 2 * D), u32), V((S // 2, 2 * D), u32), V((S // 2, 2 * D), u32), V((S // 2, 2 * D), u32),
            V((S, M), bf16), pltpu.SemaphoreType.DMA((10,))],
        compiler_params=pltpu.CompilerParams(vmem_limit_bytes=110 * 1024 * 1024),
    )(A_x.reshape(S, M), A_c_kv.reshape(S, DC), A_w_q.reshape(M * H, D), A_w_uk.reshape(DC * H, D),
      A_w_uv.reshape(DC * H, D), A_w_o.reshape(H * D, M),
      B_w_r.reshape(1, M), B_w_gate.T, B_w_up.T, B_w_down)
    return out.reshape(1, S, M)
```

```python
import functools
import math
import os
import jax
import jax.numpy as jnp
from jax import lax
import jax.experimental.pallas as pl
import jax.experimental.pallas.tpu as pltpu

S, M, DC, H, D, F, C = 2048, 640, 512, 32, 128, 1728, 8
NP = H // 2
LOG2E = math.log2(math.e)
QSCALE = (D ** -0.5) * LOG2E
MASKV = -998244352.0 * LOG2E
EPS = 1.0013580322265625e-05
BQ = 256
NB = S // BQ
CH = int(os.environ.get("CH", "4"))
f32, bf16, u32, i32 = jnp.float32, jnp.bfloat16, jnp.uint32, jnp.int32
NT = (((1,), (1,)), ((), ()))


def _rb(x):
    return x.astype(bf16).astype(f32)


def _pk(x):
    return pltpu.bitcast(x.astype(bf16), u32)


def _ld(ref, r0, r1, cs=slice(None)):
    return pltpu.bitcast(ref[r0 // 2:r1 // 2, cs], bf16)


def _dot(a, b):
    return jnp.dot(a, b, preferred_element_type=f32)


def _dot_nt(a, b):
    return lax.dot_general(a, b, NT, preferred_element_type=f32)


def body(x_hbm, c_hbm, wq_hbm, wk_hbm, wv_hbm, wo_hbm, wr_hbm, wg_hbm, wu_hbm, wd_hbm, o_hbm,
         x_p, wq_r, wk_r, wv_r, wr_v, wg_p, wu_p, wd_p, acc_v,
         xn_p, c_p, wq_p, wk_p, wv_p, wo_p, q_p, k_p, v_p, ctx_p, o_p, r_v, idx_v, rs_v, idx_s,
         sem_x, sem_w, sem_o, sem_f, sem_out):
    XS = int(os.environ.get("XS", "4"))

    def xc_cps(part):
        rs = pl.ds(0, XS * BQ // 2) if part == 0 else pl.ds(XS * BQ // 2, (NB - XS) * BQ // 2)
        return [pltpu.make_async_copy(s.bitcast(u32).at[rs], d.at[rs], sem_x.at[2 * part + n])
                for n, (s, d) in enumerate(((x_hbm, x_p), (c_hbm, c_p)))]

    def w_cps(j):
        return [pltpu.make_async_copy(s.bitcast(u32).at[:, jnp.minimum(j, NP - 1), :], d.at[j % 2], sem_w.at[3 * (j % 2) + n])
                for n, (s, d) in enumerate(((wk_hbm, wk_r), (wq_hbm, wq_r), (wv_hbm, wv_r)))]

    def wo_cp(j):
        return pltpu.make_async_copy(wo_hbm.bitcast(u32).at[pl.ds(pl.multiple_of(jnp.minimum(j, NP - 1) * D, D), D)],
                                     wo_p.at[j % 2], sem_o.at[j % 2])

    f_cps = [pltpu.make_async_copy(s.bitcast(u32), d, sem_f.at[n])
             for n, (s, d) in enumerate(((wg_hbm, wg_p), (wu_hbm, wu_p), (wd_hbm, wd_p)))]
    wr_cp = pltpu.make_async_copy(wr_hbm, wr_v, sem_f.at[3])
    idx_cp = pltpu.make_async_copy(idx_v, idx_s, sem_f.at[4])

    def out_cp(part):
        rs = pl.ds(0, (NB - 1) * BQ // 2) if part == 0 else pl.ds((NB - 1) * BQ // 2, BQ // 2)
        return pltpu.make_async_copy(o_p.at[rs], o_hbm.bitcast(u32).at[rs], sem_out.at[part])

    def unpack_w(j):
        for src, dst in ((wk_r, wk_p), (wq_r, wq_p), (wv_r, wv_p)):
            w = src[j % 2]
            dst[:, 0:D] = _pk(pltpu.bitcast(w << 16, f32))
            dst[:, D:2 * D] = _pk(pltpu.bitcast(w & jnp.uint32(0xFFFF0000), f32))

    def layernorm(i):
        r0, r1 = i * BQ, (i + 1) * BQ
        x = _ld(x_p, r0, r1).astype(f32)
        m = jnp.mean(x, axis=-1, keepdims=True)
        xc = x - m
        v = jnp.mean(xc * xc, axis=-1, keepdims=True)
        den = _rb(jnp.sqrt(_rb(_rb(v) + EPS)))
        xn_b = (_rb(x - _rb(m)) * (1.0 / den)).astype(bf16)
        xn_p[r0 // 2:r1 // 2, :] = pltpu.bitcast(xn_b, u32)
        xn = xn_b.astype(f32)
        acc_v[r0:r1, :] = x + xn
        r = jnp.sum(xn * wr_v[...].astype(f32), axis=-1, keepdims=True)
        grp = lax.broadcasted_iota(i32, (BQ, D), 0) // 8 + (i % 4) * (BQ // 8)
        lane = lax.broadcasted_iota(i32, (BQ, D), 1)
        rr = jnp.where(lane == grp, r, 0.0).reshape(BQ // 8, 8, D).sum(axis=0)
        cs = slice((i // 4) * D, (i // 4 + 1) * D)
        if i % 4 == 0:
            r_v[:, cs] = rr
        else:
            r_v[:, cs] += rr

    def all_reduce(op, red, a):
        a = red(op(a[:, :D], a[:, D:]), axis=1, keepdims=True)
        a = jnp.broadcast_to(red(jnp.broadcast_to(a, (8, D)), axis=0, keepdims=True), (8, D))
        return a

    def route():
        r = _rb(r_v[...])
        tok = (lax.broadcasted_iota(i32, (8, S // 8), 1) * 8 + lax.broadcasted_iota(i32, (8, S // 8), 0)).astype(f32)
        key = jnp.where(r != r, -jnp.inf, r)
        sub = lax.broadcasted_iota(i32, (8, D), 0)
        idxs = jnp.zeros((8, D), f32)
        rs = jnp.zeros((8, D), f32)
        for n in range(C):
            mx = all_reduce(jnp.maximum, jnp.max, key)
            idx = all_reduce(jnp.minimum, jnp.min, jnp.where(key == jnp.concatenate([mx, mx], axis=1), tok, 2.0 * S))
            hit = tok == jnp.concatenate([idx, idx], axis=1)
            key = jnp.where(hit, -jnp.inf, key)
            tok = jnp.where(hit, 2.0 * S, tok)
            idxs = jnp.where(sub == n, idx, idxs)
            rs = jnp.where(sub == n, mx, rs)
        idx_v[...] = jnp.clip(idxs.astype(i32), 0, S - 1)
        rs_v[...] = rs

    def ffn():
        sub = lax.broadcasted_iota(i32, (8, M), 0)
        xs = jnp.zeros((8, M), f32)
        idxs = [jnp.clip(idx_s[n, 0], 0, S - 1) for n in range(C)]
        for n, idx in enumerate(idxs):
            w = xn_p[pl.ds(idx // 2, 1), :]
            row = pltpu.bitcast((w >> (16 * (idx % 2)).astype(u32)) << 16, f32)
            xs = jnp.where(sub == n, row, xs)
        xs = xs.astype(bf16)
        g = _rb(_dot_nt(xs, pltpu.bitcast(wg_p[...], bf16)))
        u = _rb(_dot_nt(xs, pltpu.bitcast(wu_p[...], bf16)))
        g = _rb(g * _rb(jax.nn.sigmoid(g)))
        y = _rb(_dot((g * u).astype(bf16), pltpu.bitcast(wd_p[...], bf16)))
        y = _rb(y * _rb(jax.nn.sigmoid(rs_v[:, :1])))
        for n, idx in enumerate(idxs):
            acc_v[pl.ds(idx, 1), :] += y[n:n + 1, :]

    tri = (lax.broadcasted_iota(i32, (D, D), 1) <= lax.broadcasted_iota(i32, (D, D), 0))

    def proj_kq(i):
        r0, r1 = i * BQ, (i + 1) * BQ
        k_p[r0 // 2:r1 // 2, :] = _pk(_dot(_ld(c_p, r0, r1), pltpu.bitcast(wk_p[...], bf16)))
        q_p[r0 // 2:r1 // 2, :] = _pk(_dot(_ld(xn_p, r0, r1), pltpu.bitcast(wq_p[...], bf16)) * QSCALE)

    def proj_v(i):
        r0, r1 = i * BQ, (i + 1) * BQ
        v_p[r0 // 2:r1 // 2, :] = _pk(_dot(_ld(c_p, r0, r1), pltpu.bitcast(wv_p[...], bf16)))

    def proj(i):
        proj_kq(i)
        proj_v(i)

    def qk(i, hh):
        r0, r1 = i * BQ, (i + 1) * BQ
        cs = slice(hh * D, (hh + 1) * D)
        nt = r0 // D + 1
        q = _ld(q_p, r0, r1, cs)
        tiles = []
        for t0 in range(0, nt, CH):
            t1 = min(t0 + CH, nt)
            s = _dot_nt(q, _ld(k_p, t0 * D, t1 * D, cs))
            tiles += [s[:, t * D:(t + 1) * D] for t in range(t1 - t0)]
        tiles[-1] = jnp.concatenate([jnp.where(tri, tiles[-1][:D], MASKV), tiles[-1][D:]], axis=0)
        s1 = jnp.where(tri, _dot_nt(q[D:], _ld(k_p, r0 + D, r1, cs)), MASKV)
        mx = functools.reduce(jnp.maximum, tiles)
        mx = jnp.concatenate([mx[:D], jnp.maximum(mx[D:], s1)], axis=0)
        m = jnp.broadcast_to(jnp.max(mx, axis=-1, keepdims=True), (BQ, D))
        return tiles, s1, m

    def pv(i, hh, st):
        tiles, s1, m = st
        r0, r1 = i * BQ, (i + 1) * BQ
        cs = slice(hh * D, (hh + 1) * D)
        nt = len(tiles)
        o = l = None
        for t0 in range(0, nt, CH):
            t1 = min(t0 + CH, nt)
            ps = [jnp.exp2(s - m) for s in tiles[t0:t1]]
            lc = functools.reduce(jnp.add, ps)
            oc = _dot(jnp.concatenate([p.astype(bf16) for p in ps], axis=1), _ld(v_p, t0 * D, t1 * D, cs))
            o, l = (oc, lc) if o is None else (o + oc, l + lc)
        p1 = jnp.exp2(s1 - m[D:])
        o = jnp.concatenate([o[:D], o[D:] + _dot(p1.astype(bf16), _ld(v_p, r0 + D, r1, cs))], axis=0)
        l = jnp.sum(jnp.concatenate([l[:D], l[D:] + p1], axis=0), axis=-1, keepdims=True)
        inv = pl.reciprocal(l, approx=True)
        inv = inv * (2.0 - l * inv)
        ctx_p[r0 // 2:r1 // 2, cs] = _pk(o * inv)

    def oproj(i, j, last):
        r0, r1 = i * BQ, (i + 1) * BQ
        y = acc_v[r0:r1, :] + _dot(_ld(ctx_p, r0, r1), pltpu.bitcast(wo_p[j % 2], bf16))
        if last:
            o_p[r0 // 2:r1 // 2, :] = _pk(y)
        else:
            acc_v[r0:r1, :] = y

    def pair(j, first=False, last=False):
        if not first:
            for cp in [wo_cp(j)] + w_cps(j + 1):
                cp.wait()
        if last:
            for cp in f_cps:
                cp.wait()
            idx_cp.wait()
            ffn()
        for i in range(NB):
            if first and i == XS - 1:
                for cp in xc_cps(1) + w_cps(1):
                    cp.wait()
                for cp in [wo_cp(1)] + w_cps(2) + f_cps:
                    cp.start()
                for b in range(XS, NB):
                    layernorm(b)
                route()
            if i == NB - 1:
                if last:
                    oproj(i - 1, j, last)
                    out_cp(0).start()
                else:
                    unpack_w(j + 1)
            sa = qk(i, 0)
            sb = qk(i, 1)
            if i + 1 < NB:
                proj(i + 1)
            pv(i, 0, sa)
            if i == NB - 1 and not last:
                proj_kq(0)
            pv(i, 1, sb)
            if i > 0 and not (last and i == NB - 1):
                oproj(i - 1, j, last)
        oproj(NB - 1, j, last)
        if not last:
            proj_v(0)
        if not last:
            for cp in [wo_cp(j + 2)] + w_cps(j + 3):
                cp.start()

    first_cps = xc_cps(0) + w_cps(0)
    for cp in [first_cps[0], wr_cp] + first_cps[1:]:
        cp.start()
    first_cps[0].wait()
    wr_cp.wait()
    for cp in [wo_cp(0)] + xc_cps(1) + w_cps(1):
        cp.start()
    layernorm(0)
    for cp in first_cps[1:] + [wo_cp(0)]:
        cp.wait()
    unpack_w(0)
    for b in range(1, XS):
        layernorm(b)
    proj(0)
    pair(0, first=True)
    idx_cp.start()

    def loop_body(j, carry):
        pair(j)
        return carry
    lax.fori_loop(1, NP - 1, loop_body, None)
    pair(NP - 1, last=True)
    out_cp(1).start()
    for cp in [wo_cp(NP)] + w_cps(NP + 1):
        cp.wait()
    out_cp(0).wait()
    out_cp(1).wait()


@jax.jit
def pallas_parallel_sum__compressed_kv_cla__moe_arch_mod__prompt_kernel(
        A_x, A_c_kv, A_w_q, A_w_uk, A_w_uv, A_w_o, B_x, B_w_r, B_w_gate, B_w_up, B_w_down):
    del B_x
    V = pltpu.VMEM
    DMA = pltpu.SemaphoreType.DMA
    out = pl.pallas_call(
        body,
        in_specs=[pl.BlockSpec(memory_space=pltpu.HBM)] * 10,
        out_specs=pl.BlockSpec(memory_space=pltpu.HBM),
        out_shape=jax.ShapeDtypeStruct((S, M), bf16),
        scratch_shapes=[
            V((S // 2, M), u32), V((2, M, D), u32), V((2, DC, D), u32), V((2, DC, D), u32),
            V((1, M), bf16), V((F // 2, M), u32), V((F // 2, M), u32), V((F // 2, M), u32), V((S, M), f32),
            V((S // 2, M), u32), V((S // 2, DC), u32),
            V((M // 2, 2 * D), u32), V((DC // 2, 2 * D), u32), V((DC // 2, 2 * D), u32), V((2, D, M), u32),
            V((S // 2, 2 * D), u32), V((S // 2, 2 * D), u32), V((S // 2, 2 * D), u32), V((S // 2, 2 * D), u32),
            V((S // 2, M), u32), V((8, S // 8), f32), V((8, D), i32), V((8, D), f32), pltpu.SMEM((8, D), i32),
            DMA((4,)), DMA((6,)), DMA((2,)), DMA((5,)), DMA((2,))],
        compiler_params=pltpu.CompilerParams(vmem_limit_bytes=110 * 1024 * 1024),
    )(A_x.reshape(S, M), A_c_kv.reshape(S, DC), A_w_q, A_w_uk, A_w_uv, A_w_o.reshape(H * D, M),
      B_w_r.reshape(1, M), B_w_gate.T, B_w_up.T, B_w_down)
    return out.reshape(1, S, M)
```

```python
import functools
import math
import os
import jax
import jax.numpy as jnp
from jax import lax
import jax.experimental.pallas as pl
import jax.experimental.pallas.tpu as pltpu

S, M, DC, H, D, F, C = 2048, 640, 512, 32, 128, 1728, 8
NP = H // 2
LOG2E = math.log2(math.e)
QSCALE = (D ** -0.5) * LOG2E
MASKV = -998244352.0 * LOG2E
SAFE_GAP = 1024.0
EPS = 1.0013580322265625e-05
BQ = 256
NB = S // BQ
CH = int(os.environ.get("CH", "4"))
f32, bf16, u32, i32 = jnp.float32, jnp.bfloat16, jnp.uint32, jnp.int32
NT = (((1,), (1,)), ((), ()))


def _rb(x):
    return x.astype(bf16).astype(f32)


def _pk(x):
    return pltpu.bitcast(x.astype(bf16), u32)


def _ld(ref, r0, r1, cs=slice(None)):
    return pltpu.bitcast(ref[r0 // 2:r1 // 2, cs], bf16)


def _blk(i):
    return pl.ds(i * (BQ // 2) if isinstance(i, int) else pl.multiple_of(i * (BQ // 2), BQ // 2), BQ // 2)


def _dot(a, b):
    return jnp.dot(a, b, preferred_element_type=f32)


def _dot_nt(a, b):
    return lax.dot_general(a, b, NT, preferred_element_type=f32)


OPARTS = [(int(p[0]), int(p[1])) for p in os.environ.get("OPARTS", "48,14,01").split(",")]
R = range(7, -1, -1)
SCHED = {
    "b": "U " + " ".join(f"S{i}a S{i}b k{i} q{i-1} P{i}a v{i+1} o{i+1} P{i}b" for i in R) + " V q7 v0 o0",
    "c": "U " + " ".join(f"S{i}a S{i}b q{i-1} k{i} P{i}a o{i+1} v{i+1} P{i}b" for i in R).replace("S0a", "V q7 S0a") + " o0 v0",
    "d": "U " + " ".join(f"S{i}a S{i}b q{i-1} P{i}a k{i} o{i+1} P{i}b v{i}" for i in R).replace("S0a", "V S0a") + " q7 o0",
    "e": "U " + " ".join(f"S{i}a S{i}b q{i-1} k{i} P{i}a o{i+1} P{i}b v{i}" for i in R).replace("S0a", "V S0a") + " o0 q7",
}


def schedule(first, last):
    s = os.environ.get("SCHED", "b")
    s = SCHED.get(s, s)
    s = [t for t in s.split() if "-" not in t and "8" not in t[:2]]
    if first:
        s.remove("U")
        s.insert(s.index(os.environ.get("XAT", "P7b")), "X")
        s.insert(s.index("X") + 1, "U")
        s.remove("k7")
        s.insert(s.index("U") + 1, "k7")
    if last:
        s = [t for t in s if t[0] not in "UVkv" and t != "q7"]
        for n, (b0, _) in enumerate(OPARTS[:-1]):
            s.insert(s.index(f"o{b0}") + 1, f"D{n}")
    return s


import contextlib
def sc(name):
    return jax.named_scope(name) if os.environ.get("SCOPES") else contextlib.nullcontext()


def body(x_hbm, c_hbm, wq_hbm, wk_hbm, wv_hbm, wo_hbm, wr_hbm, wg_hbm, wu_hbm, wd_hbm, o_hbm,
         x_p, wq_r, wk_r, wv_r, wr_v, wg_p, wu_p, wd_p, acc_v,
         xn_p, c_p, wq_p, wk_p, wv_p, wo_p, q_p, k_p, v_p, ctx_p, o_p, r_v, idx_v, rs_v, idx_s, y_v, low_v,
         sem_x, sem_w, sem_o, sem_f, sem_out):
    XPARTS = [(6, 8), (0, 6)]

    def row_cp(src, dst, blocks, sem):
        rs = pl.ds(blocks[0] * BQ // 2, (blocks[1] - blocks[0]) * BQ // 2)
        return pltpu.make_async_copy(src.bitcast(u32).at[rs], dst.at[rs], sem)


    def c_cp(n):
        rs = pl.ds(n * BQ if isinstance(n, int) else pl.multiple_of(n * BQ, BQ), BQ)
        return pltpu.make_async_copy(c_hbm.bitcast(u32).at[rs], c_p.at[rs], sem_x.at[2 + n])

    x_cps = [row_cp(x_hbm, x_p, blocks, sem_x.at[n]) for n, blocks in enumerate(XPARTS)]

    def w_cps(j):
        return [pltpu.make_async_copy(s.bitcast(u32).at[:, jnp.minimum(j, NP - 1), :], d.at[j % 2], sem_w.at[3 * (j % 2) + n])
                for n, (s, d) in enumerate(((wk_hbm, wk_r), (wq_hbm, wq_r), (wv_hbm, wv_r)))]

    def wo_cp(j):
        return pltpu.make_async_copy(wo_hbm.bitcast(u32).at[pl.ds(pl.multiple_of(jnp.minimum(j, NP - 1) * D, D), D)],
                                     wo_p.at[j % 2], sem_o.at[j % 2])

    f_cps = [pltpu.make_async_copy(s.bitcast(u32), d, sem_f.at[n])
             for n, (s, d) in enumerate(((wg_hbm, wg_p), (wu_hbm, wu_p), (wd_hbm, wd_p)))]
    wr_cp = pltpu.make_async_copy(wr_hbm, wr_v, sem_f.at[3])
    idx_cp = pltpu.make_async_copy(idx_v, idx_s, sem_f.at[4])

    def out_cp(part):
        rs = pl.ds(OPARTS[part][0] * BQ // 2, (OPARTS[part][1] - OPARTS[part][0]) * BQ // 2)
        return pltpu.make_async_copy(o_p.at[rs], o_hbm.bitcast(u32).at[rs], sem_out.at[part])

    def unpack_w(j, which):
        for src, dst in dict(kv=((wk_r, wk_p), (wv_r, wv_p)), q=((wq_r, wq_p),))[which]:
            w = src[j % 2]
            dst[:, 0:D] = _pk(pltpu.bitcast(w << 16, f32))
            dst[:, D:2 * D] = _pk(pltpu.bitcast(w & jnp.uint32(0xFFFF0000), f32))

    def layernorm(i):
        r0, r1 = i * BQ, (i + 1) * BQ
        x = _ld(x_p, r0, r1).astype(f32)
        m = jnp.mean(x, axis=-1, keepdims=True)
        xc = x - m
        v = jnp.mean(xc * xc, axis=-1, keepdims=True)
        den = _rb(jnp.sqrt(_rb(_rb(v) + EPS)))
        xn_b = (_rb(x - _rb(m)) * (1.0 / den)).astype(bf16)
        xn_p[r0 // 2:r1 // 2, :] = pltpu.bitcast(xn_b, u32)
        xn = xn_b.astype(f32)
        acc_v[r0:r1, :] = x + xn
        r = jnp.sum(xn * wr_v[...].astype(f32), axis=-1, keepdims=True)
        grp = lax.broadcasted_iota(i32, (BQ, D), 0) // 8 + (i % 4) * (BQ // 8)
        lane = lax.broadcasted_iota(i32, (BQ, D), 1)
        rr = jnp.where(lane == grp, r, 0.0).reshape(BQ // 8, 8, D).sum(axis=0)
        cs = slice((i // 4) * D, (i // 4 + 1) * D)
        r_v[:, cs] += rr

    def all_reduce(op, red, a):
        a = red(op(a[:, :D], a[:, D:]), axis=1, keepdims=True)
        a = jnp.broadcast_to(red(jnp.broadcast_to(a, (8, D)), axis=0, keepdims=True), (8, D))
        return a

    def route():
        r = _rb(r_v[...])
        tok = (lax.broadcasted_iota(i32, (8, S // 8), 1) * 8 + lax.broadcasted_iota(i32, (8, S // 8), 0)).astype(f32)
        key = jnp.where(r != r, -jnp.inf, r)
        sub = lax.broadcasted_iota(i32, (8, D), 0)
        idxs = jnp.zeros((8, D), f32)
        rs = jnp.zeros((8, D), f32)
        for n in range(C):
            mx = all_reduce(jnp.maximum, jnp.max, key)
            idx = all_reduce(jnp.minimum, jnp.min, jnp.where(key == jnp.concatenate([mx, mx], axis=1), tok, 2.0 * S))
            hit = tok == jnp.concatenate([idx, idx], axis=1)
            key = jnp.where(hit, -jnp.inf, key)
            tok = jnp.where(hit, 2.0 * S, tok)
            idxs = jnp.where(sub == n, idx, idxs)
            rs = jnp.where(sub == n, mx, rs)
        idx_v[...] = jnp.clip(idxs.astype(i32), 0, S - 1)
        rs_v[...] = rs

    def ffn():
        sub = lax.broadcasted_iota(i32, (8, M), 0)
        xs = jnp.zeros((8, M), f32)
        idxs = [jnp.clip(idx_s[n, 0], 0, S - 1) for n in range(C)]
        for n, idx in enumerate(idxs):
            w = xn_p[pl.ds(idx // 2, 1), :]
            row = pltpu.bitcast((w >> (16 * (idx % 2)).astype(u32)) << 16, f32)
            xs = jnp.where(sub == n, row, xs)
        xs = xs.astype(bf16)
        g = _rb(_dot_nt(xs, pltpu.bitcast(wg_p[...], bf16)))
        u = _rb(_dot_nt(xs, pltpu.bitcast(wu_p[...], bf16)))
        g = _rb(g * _rb(jax.nn.sigmoid(g)))
        y = _rb(_dot((g * u).astype(bf16), pltpu.bitcast(wd_p[...], bf16)))
        y_v[...] = _rb(y * _rb(jax.nn.sigmoid(rs_v[:, :1])))
        scatter()

    def scatter():
        for n in range(C):
            acc_v[pl.ds(jnp.clip(idx_s[n, 0], 0, S - 1), 1), :] += y_v[n:n + 1, :]

    tri = (lax.broadcasted_iota(i32, (D, D), 1) <= lax.broadcasted_iota(i32, (D, D), 0))

    def proj_k(i):
        k_p[_blk(i), :] = _pk(_dot(pltpu.bitcast(c_p[_blk(i), :], bf16), pltpu.bitcast(wk_p[...], bf16)))

    def proj_q(i):
        q_p[_blk(i), :] = _pk(_dot(pltpu.bitcast(xn_p[_blk(i), :], bf16), pltpu.bitcast(wq_p[...], bf16)) * QSCALE)

    def proj_v(i):
        v_p[_blk(i), :] = _pk(_dot(pltpu.bitcast(c_p[_blk(i), :], bf16), pltpu.bitcast(wv_p[...], bf16)))

    def proj(i):
        proj_k(i)
        proj_q(i)
        proj_v(i)

    class Attn:
        def __init__(self, i, hh):
            self.r0, self.r1, self.hh = i * BQ, (i + 1) * BQ, hh
            self.cs = slice(hh * D, (hh + 1) * D)
            self.nt = self.r0 // D + 1
            self.chunks = [(t, min(t + CH, self.nt)) for t in range(0, self.nt, CH)]
            self.ns = self.ne = self.np_ = 0
            self.s, self.p = [], []
            self.mx = self.l = self.o = None

        def scores(self):
            r0, r1, cs = self.r0, self.r1, self.cs
            t0, t1 = self.chunks[self.ns]
            self.ns += 1
            s = _dot_nt(_ld(q_p, r0, r1, cs), _ld(k_p, t0 * D, t1 * D, cs))
            tiles = [s[:, t * D:(t + 1) * D] for t in range(t1 - t0)]
            if t1 == self.nt:
                tiles[-1] = jnp.concatenate([jnp.where(tri, tiles[-1][:D], MASKV), tiles[-1][D:]], axis=0)
            self.s.append(tiles)
            mx = functools.reduce(jnp.maximum, ([] if self.mx is None else [self.mx]) + tiles)
            if t1 == self.nt:
                self.s1 = jnp.where(tri, _dot_nt(_ld(q_p, r0 + D, r1, cs), _ld(k_p, r0 + D, r1, cs)), MASKV)
                mx = jnp.concatenate([mx[:D], jnp.maximum(mx[D:], self.s1)], axis=0)
                mx = jnp.broadcast_to(jnp.max(mx, axis=-1, keepdims=True), (BQ, D))
                low_v[...] = jnp.minimum(low_v[...], mx.reshape(BQ // 8, 8, D).min(axis=0))
            self.mx = mx

        def exp(self):
            while self.ns < len(self.chunks):
                self.scores()
            ps = [jnp.exp2(s - self.mx) for s in self.s[self.ne]]
            self.ne += 1
            self.p.append(jnp.concatenate(ps, axis=1).astype(bf16))
            l = functools.reduce(jnp.add, ([] if self.l is None else [self.l]) + ps)
            if self.ne == len(self.chunks):
                p1 = jnp.exp2(self.s1 - self.mx[D:])
                self.p1 = p1.astype(bf16)
                l = jnp.sum(jnp.concatenate([l[:D], l[D:] + p1], axis=0), axis=-1, keepdims=True)
                inv = pl.reciprocal(l, approx=True)
                l = inv * (2.0 - l * inv)
            self.l = l

        def pv(self):
            r0, r1, cs = self.r0, self.r1, self.cs
            if self.ne == self.np_:
                self.exp()
            t0, t1 = self.chunks[self.np_]
            p = self.p[self.np_]
            o = _dot(p, _ld(v_p, t0 * D, t1 * D, cs))
            self.np_ += 1
            if self.o is not None:
                o = self.o + o
            self.o = o
            if t1 == self.nt:
                o = jnp.concatenate([o[:D], o[D:] + _dot(self.p1, _ld(v_p, r0 + D, r1, cs))], axis=0)
                ctx_p[r0 // 2:r1 // 2, cs] = _pk(o * self.l)

        def run(self, op, n):
            fn, cnt = dict(S=(self.scores, "ns"), E=(self.exp, "ne"), P=(self.pv, "np_"))[op]
            while n > 0 and dict(ns=self.ns, ne=self.ne, np_=self.np_)[cnt] < len(self.chunks):
                fn()
                n -= 1

    def oproj(i, j, last):
        r0, r1 = i * BQ, (i + 1) * BQ
        y = acc_v[r0:r1, :] + _dot(_ld(ctx_p, r0, r1), pltpu.bitcast(wo_p[j % 2], bf16))
        if last:
            o_p[r0 // 2:r1 // 2, :] = _pk(y)
        else:
            acc_v[r0:r1, :] = y

    def pair(j, first=False, last=False):
        if not first:
            with sc("w_top"):
                for cp in [wo_cp(j)] + w_cps(j + 1):
                    cp.wait()
        st = {}
        for tk in schedule(first, last):
            op, i = tk[0], int(tk[1]) if len(tk) > 1 else None
            if first and tk in os.environ.get("MARK", "").split(","):
                with sc("m_" + tk):
                    rs_v[:, :] = rs_v[:, :] + 0.0
            if op in "SEP":
                if tk[1:3] not in st:
                    st[tk[1:3]] = Attn(i, "ab".index(tk[2]))
                st[tk[1:3]].run(op, int(tk[3:] or 99))
            elif op in "kqv":
                dict(k=proj_k, q=proj_q, v=proj_v)[op](i)
            elif op == "o":
                oproj(i, j, last)
            elif op == "U":
                unpack_w(j + 1, "kv")
            elif op == "V":
                unpack_w(j + 1, "q")
            elif op == "X":
                with sc("w_X"):
                    for cp in [x_cps[1], wo_cp(0)] + w_cps(1):
                        cp.wait()
                for cp in f_cps + [wo_cp(1)] + w_cps(2):
                    cp.start()
                for b in reversed(range(*XPARTS[1])):
                    layernorm(b)
                route()
            elif op == "D":
                out_cp(i).start()
        if not last:
            for cp in [wo_cp(j + 2)] + w_cps(j + 3) + ([idx_cp] if first else []):
                cp.start()

    for cp in w_cps(0) + [c_cp(0)]:
        cp.start()
    r_v[...] = jnp.zeros_like(r_v)
    low_v[...] = jnp.zeros_like(low_v)
    with sc("w_w0"):
        for cp in w_cps(0):
            cp.wait()
    for cp in [c_cp(1), c_cp(2), c_cp(3), x_cps[0], wr_cp]:
        cp.start()
    unpack_w(0, "kv")
    unpack_w(0, "q")

    def kv_body(n, carry):
        with sc("w_c"):
            c_cp(n).wait()
        for b in (2 * n, 2 * n + 1):
            proj_k(b)
            proj_v(b)
        return carry
    lax.fori_loop(0, 3, kv_body, None)
    with sc("w_x0"):
        for cp in [c_cp(3), x_cps[0], wr_cp]:
            cp.wait()
    for cp in [x_cps[1], wo_cp(0)] + w_cps(1):
        cp.start()
    layernorm(7)
    for b in (6, 7):
        proj_k(b)
        proj_v(b)
    proj_q(7)
    layernorm(6)

    def loop_body(j, carry):
        pair(j)
        return carry
    PEEL = os.environ.get("PEEL", "1")
    if PEEL in "1f":
        pair(0, first=True)
    if PEEL in "10":
        lax.fori_loop(1, NP - 1, loop_body, None)
    if PEEL in "1l":
        for cp in f_cps + [idx_cp]:
            cp.wait()
        with sc("ffn"):
            ffn()
        pair(NP - 1, last=True)
    out_cp(len(OPARTS) - 1).start()
    for cp in [wo_cp(NP)] + w_cps(NP + 1):
        cp.wait()
    with sc("w_out"):
        for n in range(len(OPARTS)):
            out_cp(n).wait()

    @pl.when(jnp.min(low_v[...]) < MASKV + SAFE_GAP)
    def _():
        def rows(i):
            return pl.ds(pl.multiple_of(i * BQ, BQ), BQ)

        @pl.loop(0, NB)
        def _(i):
            acc_v[rows(i), :] = (pltpu.bitcast(x_p[_blk(i), :], bf16).astype(f32)
                                 + pltpu.bitcast(xn_p[_blk(i), :], bf16).astype(f32))
        scatter()

        @pl.loop(0, NP)
        def _(j):
            cps = [wo_cp(j)] + w_cps(j)
            for cp in cps:
                cp.start()
            for cp in cps:
                cp.wait()
            unpack_w(j, "kv")
            unpack_w(j, "q")

            @pl.loop(0, NB)
            def _(i):
                proj_k(i)
                proj_v(i)
                proj_q(i)

            @pl.loop(0, NB)
            def _(i):
                keep = (lax.broadcasted_iota(i32, (BQ, S), 1) - lax.broadcasted_iota(i32, (BQ, S), 0)) <= i * BQ
                for cs in (slice(0, D), slice(D, 2 * D)):
                    sc_ = jnp.where(keep, _dot_nt(pltpu.bitcast(q_p[_blk(i), cs], bf16), _ld(k_p, 0, S, cs)), MASKV)
                    p = jnp.exp2(sc_ - jnp.max(sc_, axis=-1, keepdims=True))
                    o = _dot(p.astype(bf16), _ld(v_p, 0, S, cs))
                    ctx_p[_blk(i), cs] = _pk(o / jnp.sum(p, axis=-1, keepdims=True))
                acc_v[rows(i), :] += _dot(pltpu.bitcast(ctx_p[_blk(i), :], bf16), pltpu.bitcast(wo_p[j % 2], bf16))

        @pl.loop(0, NB)
        def _(i):
            o_p[_blk(i), :] = _pk(acc_v[rows(i), :])
        for n in range(len(OPARTS)):
            out_cp(n).start()
        for n in range(len(OPARTS)):
            out_cp(n).wait()


@jax.jit
def pallas_parallel_sum__compressed_kv_cla__moe_arch_mod__prompt_kernel(
        A_x, A_c_kv, A_w_q, A_w_uk, A_w_uv, A_w_o, B_x, B_w_r, B_w_gate, B_w_up, B_w_down):
    del B_x
    V = pltpu.VMEM
    DMA = pltpu.SemaphoreType.DMA
    out = pl.pallas_call(
        body,
        in_specs=[pl.BlockSpec(memory_space=pltpu.HBM)] * 10,
        out_specs=pl.BlockSpec(memory_space=pltpu.HBM),
        out_shape=jax.ShapeDtypeStruct((S, M), bf16),
        scratch_shapes=[
            V((S // 2, M), u32), V((2, M, D), u32), V((2, DC, D), u32), V((2, DC, D), u32),
            V((1, M), bf16), V((F // 2, M), u32), V((F // 2, M), u32), V((F // 2, M), u32), V((S, M), f32),
            V((S // 2, M), u32), V((S // 2, DC), u32),
            V((M // 2, 2 * D), u32), V((DC // 2, 2 * D), u32), V((DC // 2, 2 * D), u32), V((2, D, M), u32),
            V((S // 2, 2 * D), u32), V((S // 2, 2 * D), u32), V((S // 2, 2 * D), u32), V((S // 2, 2 * D), u32),
            V((S // 2, M), u32), V((8, S // 8), f32), V((8, D), i32), V((8, D), f32), pltpu.SMEM((8, D), i32), V((8, M), f32), V((8, D), f32),
            DMA((16,)), DMA((6,)), DMA((2,)), DMA((5,)), DMA((len(OPARTS),))],
        compiler_params=pltpu.CompilerParams(vmem_limit_bytes=110 * 1024 * 1024, flags={k: True for k in os.environ.get('FLAGS', '').split(',') if k}),
    )(A_x.reshape(S, M), A_c_kv.reshape(S, DC), A_w_q, A_w_uk, A_w_uv, A_w_o.reshape(H * D, M),
      B_w_r.reshape(1, M), B_w_gate.T, B_w_up.T, B_w_down)
    return out.reshape(1, S, M)
```

```python
import functools
import math

import jax
import jax.numpy as jnp
from jax import lax
import jax.experimental.pallas as pl
import jax.experimental.pallas.tpu as pltpu

S, M, DC, H, D, F, C = 2048, 640, 512, 32, 128, 1728, 8
NP = H // 2
BQ = 256
NB = S // BQ
CH = 4
LOG2E = math.log2(math.e)
QSCALE = (D ** -0.5) * LOG2E
MASKV = -998244352.0 * LOG2E
SAFE_GAP = 1024.0
EPS = 1.0013580322265625e-05
OUT_PARTS = ((4, 8), (1, 4), (0, 1))
f32, bf16, u32, i32 = jnp.float32, jnp.bfloat16, jnp.uint32, jnp.int32

SCHED = ("U S7b q6 P7b S7a P7a S6b v7 P6b q5 S6a k7 P6a S5b v6 P5b o7 q4 S5a k6 P5a o6 S4b v5 P4b q3 S4a k5 "
         "P4a S3b v4 P3b o5 S3a q2 k4 P3a o4 S2b S2a v3 P2b k3 q1 P2a o3 S1b v2 q0 V S1a k2 P1b P1a o2 S0b v1 "
         "P0b S0a q7 P0a o1 k1 v0 k0 o0 ")
FSCHED = ("S7b q6 S7a P7a X U k7 N3 P7b S6a S6b k6 q5 N2 o7 P6a S5a v7 N1 P6b S5b q4 k5 v6 N0 P5a R P5b o6 S4b "
          "S4a k4 v5 q3 P4a P4b S3a S3b k3 o5 q2 P3a P3b v4 S2a S2b o4 k2 q1 P2a P2b v2 v3 o3 S1a S1b k1 q0 P1a "
          "o2 P1b S0a S0b k0 P0a v1 o1 P0b V q7 v0 o0 ")
LSCHED = ("S7a S7b q6 P7a P7b S6b S6a q5 P6a o7 P6b S5a q4 S5b P5a P5b o6 S4a S4b q3 P4a S3b o5 P4b S3a q2 P3a "
          "o4 P3b S2a S2b P2a D0 q1 P2b S1a S1b o3 q0 P1a o2 P1b S0a S0b o1 P0a P0b D1 o0 ")


def _rb(x):
    return x.astype(bf16).astype(f32)


def _pk(x):
    return pltpu.bitcast(x.astype(bf16), u32)


def _unpk(w):
    return pltpu.bitcast(w, bf16)


def _ld(ref, r0, r1, cs):
    return _unpk(ref[r0 // 2:r1 // 2, cs])


def _rows(i, n):
    return pl.ds(i * n if isinstance(i, int) else pl.multiple_of(i * n, n), n)


def _blk(i):
    return _rows(i, BQ // 2)


def _dot(a, b):
    return jnp.dot(a, b, preferred_element_type=f32)


def _dot_nt(a, b):
    return lax.dot_general(a, b, (((1,), (1,)), ((), ())), preferred_element_type=f32)


def _body(x_hbm, c_hbm, wq_hbm, wk_hbm, wv_hbm, wo_hbm, wr_hbm, wg_hbm, wu_hbm, wd_hbm, o_hbm,
          x_p, c_p, wq_r, wk_r, wv_r, wo_p, wr_v, wg_p, wu_p, wd_p,
          xn_p, wq_p, wk_p, wv_p, q_p, k_p, v_p, ctx_p, acc_v, o_p,
          r_v, idx_v, rs_v, idx_s, y_v, low_v,
          sem_x, sem_w, sem_o, sem_f, sem_out):
    def rows_cp(src, dst, rows, sem):
        return pltpu.make_async_copy(src.bitcast(u32).at[rows], dst.at[rows], sem)

    def c_cp(n):
        return rows_cp(c_hbm, c_p, _rows(n, BQ), sem_x.at[n])

    def x_cp(n):
        return rows_cp(x_hbm, x_p, _blk(NB - 1 - n), sem_x.at[4 + n])

    x_rest = rows_cp(x_hbm, x_p, pl.ds(0, 3 * BQ // 2), sem_x.at[9])

    def w_cps(j):
        return [pltpu.make_async_copy(s.bitcast(u32).at[:, jnp.minimum(j, NP - 1), :], d.at[j & 1],
                                      sem_w.at[3 * (j & 1) + n])
                for n, (s, d) in enumerate(((wk_hbm, wk_r), (wq_hbm, wq_r), (wv_hbm, wv_r)))]

    def wo_cp(j):
        return pltpu.make_async_copy(wo_hbm.bitcast(u32).at[_rows(jnp.minimum(j, NP - 1), D)],
                                     wo_p.at[j & 1], sem_o.at[j & 1])

    f_cps = [pltpu.make_async_copy(s.bitcast(u32), d, sem_f.at[n])
             for n, (s, d) in enumerate(((wg_hbm, wg_p), (wu_hbm, wu_p), (wd_hbm, wd_p)))]
    wr_cp = pltpu.make_async_copy(wr_hbm, wr_v, sem_f.at[3])
    idx_cp = pltpu.make_async_copy(idx_v, idx_s, sem_f.at[4])

    def out_cp(n):
        b0, b1 = OUT_PARTS[n]
        rows = pl.ds(b0 * BQ // 2, (b1 - b0) * BQ // 2)
        return pltpu.make_async_copy(o_p.at[rows], o_hbm.bitcast(u32).at[rows], sem_out.at[n])

    def start(cps):
        for cp in cps:
            cp.start()

    def wait(cps):
        for cp in cps:
            cp.wait()

    def unpack_w(j, bufs):
        for src, dst in bufs:
            w = src[j & 1]
            dst[:, :D] = _pk(pltpu.bitcast(w << 16, f32))
            dst[:, D:] = _pk(pltpu.bitcast(w & jnp.uint32(0xFFFF0000), f32))

    w_kv, w_q = ((wk_r, wk_p), (wv_r, wv_p)), ((wq_r, wq_p),)

    def proj_k(i):
        k_p[_blk(i), :] = _pk(_dot(_unpk(c_p[_blk(i), :]), _unpk(wk_p[...])))

    def proj_v(i):
        v_p[_blk(i), :] = _pk(_dot(_unpk(c_p[_blk(i), :]), _unpk(wv_p[...])))

    def proj_q(i):
        q_p[_blk(i), :] = _pk(_dot(_unpk(xn_p[_blk(i), :]), _unpk(wq_p[...])) * QSCALE)

    def proj_o(i, j, last):
        y = acc_v[_rows(i, BQ), :] + _dot(_unpk(ctx_p[_blk(i), :]), _unpk(wo_p[j & 1]))
        if last:
            o_p[_blk(i), :] = _pk(y)
        else:
            acc_v[_rows(i, BQ), :] = y

    def layernorm(i):
        x = _unpk(x_p[_blk(i), :]).astype(f32)
        m = jnp.mean(x, axis=-1, keepdims=True)
        xc = x - m
        v = jnp.mean(xc * xc, axis=-1, keepdims=True)
        den = _rb(jnp.sqrt(_rb(_rb(v) + EPS)))
        xn_b = (_rb(x - _rb(m)) * (1.0 / den)).astype(bf16)
        xn_p[_blk(i), :] = pltpu.bitcast(xn_b, u32)
        xn = xn_b.astype(f32)
        acc_v[_rows(i, BQ), :] = x + xn
        r = jnp.sum(xn * wr_v[...].astype(f32).reshape(1, M), axis=-1, keepdims=True)
        grp = lax.broadcasted_iota(i32, (BQ, D), 0) // 8
        lane = lax.broadcasted_iota(i32, (BQ, D), 1) - (i & 3) * (BQ // 8)
        r_v[i >> 2] += jnp.where(lane == grp, r, 0.0).reshape(BQ // 8, 8, D).sum(axis=0)

    def all_reduce(op, red, a):
        a = red(op(a[:, :D], a[:, D:]), axis=1, keepdims=True)
        return jnp.broadcast_to(red(jnp.broadcast_to(a, (8, D)), axis=0, keepdims=True), (8, D))

    def route():
        r = _rb(jnp.concatenate([r_v[0], r_v[1]], axis=1))
        tok = (lax.broadcasted_iota(i32, (8, S // 8), 1) * 8 + lax.broadcasted_iota(i32, (8, S // 8), 0)).astype(f32)
        key = jnp.where(r != r, -jnp.inf, r)
        sub = lax.broadcasted_iota(i32, (8, D), 0)
        idxs = jnp.zeros((8, D), f32)
        rs = jnp.zeros((8, D), f32)
        for n in range(C):
            mx = all_reduce(jnp.maximum, jnp.max, key)
            idx = all_reduce(jnp.minimum, jnp.min, jnp.where(key == jnp.concatenate([mx, mx], axis=1), tok, 2.0 * S))
            hit = tok == jnp.concatenate([idx, idx], axis=1)
            key = jnp.where(hit, -jnp.inf, key)
            tok = jnp.where(hit, 2.0 * S, tok)
            idxs = jnp.where(sub == n, idx, idxs)
            rs = jnp.where(sub == n, mx, rs)
        idx_v[...] = idxs.astype(i32)
        rs_v[...] = rs

    def token(n):
        return jnp.clip(idx_s[n, 0], 0, S - 1)

    def ffn():
        sub = lax.broadcasted_iota(i32, (8, M), 0)
        xs = jnp.zeros((8, M), f32)
        for n in range(C):
            idx = token(n)
            w = xn_p[pl.ds(idx >> 1, 1), :]
            xs = jnp.where(sub == n, pltpu.bitcast((w >> (16 * (idx & 1)).astype(u32)) << 16, f32), xs)
        xs = xs.astype(bf16)
        g = _rb(_dot_nt(xs, _unpk(wg_p[...])))
        u = _rb(_dot_nt(xs, _unpk(wu_p[...])))
        g = _rb(g * _rb(jax.nn.sigmoid(g)))
        y = _rb(_dot((g * u).astype(bf16), _unpk(wd_p[...])))
        y_v[...] = _rb(y * _rb(jax.nn.sigmoid(rs_v[:, :1])))

    def scatter():
        for n in range(C):
            acc_v[pl.ds(token(n), 1), :] += y_v[n:n + 1, :]

    tri = lax.broadcasted_iota(i32, (D, D), 1) <= lax.broadcasted_iota(i32, (D, D), 0)

    def chunks(i):
        nt = i * BQ // D + 1
        return [(t, min(t + CH, nt)) for t in range(0, nt, CH)]

    def scores(i, hh):
        r0, r1 = i * BQ, (i + 1) * BQ
        cs = slice(hh * D, (hh + 1) * D)
        tiles = []
        for t0, t1 in chunks(i):
            s = _dot_nt(_ld(q_p, r0, r1, cs), _ld(k_p, t0 * D, t1 * D, cs))
            tiles += [s[:, t * D:(t + 1) * D] for t in range(t1 - t0)]
        tiles[-1] = jnp.concatenate([jnp.where(tri, tiles[-1][:D], MASKV), tiles[-1][D:]], axis=0)
        mx = functools.reduce(jnp.maximum, tiles)
        s1 = jnp.where(tri, _dot_nt(_ld(q_p, r0 + D, r1, cs), _ld(k_p, r0 + D, r1, cs)), MASKV)
        mx = jnp.concatenate([mx[:D], jnp.maximum(mx[D:], s1)], axis=0)
        mx = jnp.broadcast_to(jnp.max(mx, axis=-1, keepdims=True), (BQ, D))
        low_v[...] = jnp.minimum(low_v[...], mx.reshape(BQ // 8, 8, D).min(axis=0))
        return tiles, s1, mx

    def context(i, hh, tiles, s1, mx):
        r0, r1 = i * BQ, (i + 1) * BQ
        cs = slice(hh * D, (hh + 1) * D)
        o, l = None, []
        for t0, t1 in chunks(i):
            ps = [jnp.exp2(s - mx) for s in tiles[t0:t1]]
            p = jnp.concatenate(ps, axis=1).astype(bf16)
            l = [functools.reduce(jnp.add, l + ps)]
            if t1 == len(tiles):
                p1 = jnp.exp2(s1 - mx[D:])
                p1b = p1.astype(bf16)
                l = jnp.sum(jnp.concatenate([l[0][:D], l[0][D:] + p1], axis=0), axis=-1, keepdims=True)
                inv = pl.reciprocal(l, approx=True)
                inv = inv * (2.0 - l * inv)
            oc = _dot(p, _ld(v_p, t0 * D, t1 * D, cs))
            o = oc if o is None else o + oc
        o = jnp.concatenate([o[:D], o[D:] + _dot(p1b, _ld(v_p, r0 + D, r1, cs))], axis=0)
        ctx_p[_blk(i), cs] = _pk(o * inv)

    def pair(j, sched, first=False, last=False):
        if not first:
            wait([wo_cp(j)] + w_cps(j + 1))
        st = {}
        for tk in sched.split():
            op, i = tk[0], int(tk[1]) if len(tk) > 1 else None
            if op == "S":
                st[tk[1:]] = scores(i, "ab".index(tk[2]))
            elif op == "P":
                context(i, "ab".index(tk[2]), *st[tk[1:]])
            elif op == "q":
                proj_q(i)
            elif op == "k":
                proj_k(i)
            elif op == "v":
                proj_v(i)
            elif op == "o":
                proj_o(i, j, last)
            elif op == "U":
                unpack_w(j + 1, w_kv)
            elif op == "V":
                unpack_w(j + 1, w_q)
            elif op == "X":
                wait([x_rest, wo_cp(0)] + w_cps(1))
                start(f_cps + [wo_cp(1)] + w_cps(2))
            elif op == "N":
                layernorm(i)
            elif op == "R":
                route()
            elif op == "D":
                out_cp(i).start()
        if not last:
            start([wo_cp(j + 2)] + w_cps(j + 3) + ([idx_cp] if first else []))

    wk0, wq0, wv0 = w_cps(0)
    start([x_cp(0), wr_cp, wk0, wv0, c_cp(0)])
    r_v[...] = jnp.zeros_like(r_v)
    low_v[...] = jnp.zeros_like(low_v)
    wait([x_cp(0), wr_cp])
    x_cp(1).start()
    layernorm(NB - 1)
    wait([wk0, wv0])
    wq0.start()
    unpack_w(0, w_kv)

    def first_kv(n):
        for b in (2 * n, 2 * n + 1):
            proj_k(b)
            proj_v(b)

    @pl.loop(0, 3)
    def _(n):
        wait([c_cp(n), x_cp(n + 1)])
        start([c_cp(n + 1), x_cp(n + 2)])
        first_kv(n)
        layernorm(NB - 2 - n)

    start([wo_cp(0), x_rest] + w_cps(1))
    wait([c_cp(3), x_cp(4), wq0])
    unpack_w(0, w_q)
    first_kv(3)
    proj_q(NB - 1)
    pair(0, FSCHED, first=True)

    @pl.loop(1, NP - 1)
    def _(j):
        pair(j, SCHED)

    wait(f_cps + [idx_cp])
    ffn()
    scatter()
    pair(NP - 1, LSCHED, last=True)
    out_cps = [out_cp(n) for n in range(len(OUT_PARTS))]
    out_cps[-1].start()
    wait([wo_cp(NP)] + w_cps(NP + 1) + out_cps)

    @pl.when(jnp.min(low_v[...]) < MASKV + SAFE_GAP)
    def _():
        @pl.loop(0, NB)
        def _(i):
            acc_v[_rows(i, BQ), :] = _unpk(x_p[_blk(i), :]).astype(f32) + _unpk(xn_p[_blk(i), :]).astype(f32)
        scatter()

        @pl.loop(0, NP)
        def _(j):
            cps = [wo_cp(j)] + w_cps(j)
            start(cps)
            wait(cps)
            unpack_w(j, w_kv + w_q)

            @pl.loop(0, NB)
            def _(i):
                proj_k(i)
                proj_v(i)
                proj_q(i)

            @pl.loop(0, NB)
            def _(i):
                keep = lax.broadcasted_iota(i32, (BQ, S), 1) - lax.broadcasted_iota(i32, (BQ, S), 0) <= i * BQ
                for cs in (slice(0, D), slice(D, 2 * D)):
                    s = jnp.where(keep, _dot_nt(_unpk(q_p[_blk(i), cs]), _ld(k_p, 0, S, cs)), MASKV)
                    p = jnp.exp2(s - jnp.max(s, axis=-1, keepdims=True))
                    o = _dot(p.astype(bf16), _ld(v_p, 0, S, cs))
                    ctx_p[_blk(i), cs] = _pk(o / jnp.sum(p, axis=-1, keepdims=True))
                proj_o(i, j, False)

        @pl.loop(0, NB)
        def _(i):
            o_p[_blk(i), :] = _pk(acc_v[_rows(i, BQ), :])
        start(out_cps)
        wait(out_cps)


@jax.jit
def pallas_parallel_sum__compressed_kv_cla__moe_arch_mod__prompt_kernel(
    A_x: jax.Array,
    A_c_kv: jax.Array,
    A_w_q: jax.Array,
    A_w_uk: jax.Array,
    A_w_uv: jax.Array,
    A_w_o: jax.Array,
    B_x: jax.Array,
    B_w_r: jax.Array,
    B_w_gate: jax.Array,
    B_w_up: jax.Array,
    B_w_down: jax.Array,
):
    del B_x
    V = pltpu.VMEM
    DMA = pltpu.SemaphoreType.DMA
    out = pl.pallas_call(
        _body,
        in_specs=[pl.BlockSpec(memory_space=pltpu.HBM)] * 10,
        out_specs=pl.BlockSpec(memory_space=pltpu.HBM),
        out_shape=jax.ShapeDtypeStruct((S, M), bf16),
        scratch_shapes=[
            V((S // 2, M), u32), V((S // 2, DC), u32),
            V((2, M, D), u32), V((2, DC, D), u32), V((2, DC, D), u32), V((2, D, M), u32),
            V((M,), bf16), V((F // 2, M), u32), V((F // 2, M), u32), V((F // 2, M), u32),
            V((S // 2, M), u32),
            V((M // 2, 2 * D), u32), V((DC // 2, 2 * D), u32), V((DC // 2, 2 * D), u32),
            V((S // 2, 2 * D), u32), V((S // 2, 2 * D), u32), V((S // 2, 2 * D), u32),
            V((S // 2, 2 * D), u32),
            V((S, M), f32), V((S // 2, M), u32),
            V((2, 8, D), f32), V((8, D), i32), V((8, D), f32), pltpu.SMEM((8, D), i32),
            V((8, M), f32), V((8, D), f32),
            DMA((10,)), DMA((6,)), DMA((2,)), DMA((5,)), DMA((len(OUT_PARTS),)),
        ],
        compiler_params=pltpu.CompilerParams(vmem_limit_bytes=110 * 1024 * 1024),
    )(A_x.reshape(S, M), A_c_kv.reshape(S, DC), A_w_q, A_w_uk, A_w_uv, A_w_o.reshape(H * D, M),
      B_w_r, B_w_gate.T, B_w_up.T, B_w_down)
    return out.reshape(1, S, M)
```
